```python
import os as _os
_os.environ.setdefault('JAX_PLATFORMS', 'cpu')
import jax
import jax.numpy as jnp

def _softmax(x, axis=-1):
    return jax.nn.softmax(x, axis=axis)

def _gelu(x):
    return jax.nn.gelu(x, approximate=True)

def _silu(x):
    return jax.nn.silu(x)

def _sigmoid(x):
    return jax.nn.sigmoid(x)

def _layernorm(x, axis=-1, eps=1e-05):
    m = jnp.mean(x, axis=axis, keepdims=True)
    v = jnp.var(x, axis=axis, keepdims=True)
    return (x - m) / jnp.sqrt(v + eps)

def _scatter_add(tgt, idx, src, axis=0):
    return tgt.at[idx].add(src)

def _segment_sum(src, seg, n):
    return jax.ops.segment_sum(src, seg, n)

class _Rng:

    def __init__(self, key):
        self._k = key

    def _next(self):
        self._k, sub = jax.random.split(self._k)
        return sub

    def normal(self, shape):
        return jax.random.normal(self._next(), shape, dtype=jnp.bfloat16)

    def randint(self, lo, hi, shape):
        return jax.random.randint(self._next(), shape, lo, hi, dtype=jnp.int32)

    def uniform(self, shape, lo=0.0, hi=1.0):
        return jax.random.uniform(self._next(), shape, jnp.bfloat16, lo, hi)

    def permutation(self, n):
        return jax.random.permutation(self._next(), n)
kernel_name = 'adaLN_cond__memory_aug_recurrent_mem_tr__moe_arch_mod__prompt'

def setup_inputs():
    _rng = _Rng(jax.random.key(int.from_bytes(__import__("os").urandom(4), "little")))
    _w = lambda a: (lambda t: t.astype(jnp.bfloat16) if jnp.issubdtype(t.dtype, jnp.floating) else t)(jnp.asarray(a))

    def _A_setup():
        B, S, Dm = (1, 2048, 448)
        H, Dh = (16, 256)
        M, seg = (8, 32)
        seg = min(seg, S)
        S = S // seg * seg
        return {'x': _w((lambda *s: _rng.normal(s) * 0.05)(B, S, Dm)), 'mem0': _w((lambda *s: _rng.normal(s) * 0.4)(B, M, Dm)), 'Wq': _w((lambda *s: _rng.normal(s) * 1.6)(Dm, H, Dh) * Dm ** (-0.5)), 'Wk': _w((lambda *s: _rng.normal(s) * 1.6)(Dm, H, Dh) * Dm ** (-0.5)), 'Wv': _w((lambda *s: _rng.normal(s) * 0.4)(Dm, H, Dh) * Dm ** (-0.5)), 'Wo': _w((lambda *s: _rng.normal(s) * 0.4)(H, Dh, Dm) * (H * Dh) ** (-0.5)), 'seg_len': seg}
    _A_in = _A_setup()

    def _B_setup():
        B, S, D, F, C = (1, 2048, 448, 1792, 1)
        return {'x': _w((lambda *s: _rng.normal(s) * 0.05)(B, S, D)), 'w_r': _w((lambda *s: _rng.normal(s) * 0.05)(D)), 'w_gate': _w((lambda *s: _rng.normal(s) * 0.05)(D, F)), 'w_up': _w((lambda *s: _rng.normal(s) * 0.05)(D, F)), 'w_down': _w((lambda *s: _rng.normal(s) * 0.05)(F, D))}
    _B_in = _B_setup()
    return {'A_x': _A_in['x'], 'A_mem0': _A_in['mem0'], 'A_Wq': _A_in['Wq'], 'A_Wk': _A_in['Wk'], 'A_Wv': _A_in['Wv'], 'A_Wo': _A_in['Wo'], 'A_seg_len': _A_in['seg_len'], 'B_x': _B_in['x'], 'B_w_r': _B_in['w_r'], 'B_w_gate': _B_in['w_gate'], 'B_w_up': _B_in['w_up'], 'B_w_down': _B_in['w_down'], 'c': _w((lambda *s: _rng.normal(s) * 0.05)(1, 448) * 8.0), 'w_mod': _w((lambda *s: _rng.normal(s) * 0.05)(448, 6 * 448) * 448 ** (-0.5) * 8.0)}

def reference(A_x, A_mem0, A_Wq, A_Wk, A_Wv, A_Wo, A_seg_len, B_x, B_w_r, B_w_gate, B_w_up, B_w_down, c, w_mod):

    def _A_ref(x, mem0, Wq, Wk, Wv, Wo, seg_len):
        B, S, Dm = x.shape
        H, Dh = (Wq.shape[1], Wq.shape[2])
        M = mem0.shape[1]
        scale = Dh ** (-0.5)
        n_seg = S // seg_len
        L = M + seg_len
        idx = jnp.arange(L)
        mask = (idx[:, None] < M) | (idx[:, None] >= idx[None, :])
        mem = mem0
        outs = []
        for s in range(n_seg):
            xs = x[:, s * seg_len:(s + 1) * seg_len, :].copy()
            h = jnp.concatenate([mem, xs], axis=1)
            q = jnp.einsum('btd,dhe->bhte', h, Wq)
            k = jnp.einsum('btd,dhe->bhte', h, Wk)
            v = jnp.einsum('btd,dhe->bhte', h, Wv)
            scores = jnp.einsum('bhqe,bhke->bhqk', q, k) * scale
            scores = jnp.where(mask[None, None], scores, -1000000000.0)
            p = _softmax(scores, axis=-1)
            o = jnp.einsum('bhqk,bhke->bhqe', p, v)
            o = jnp.einsum('bhte,hed->btd', o, Wo)
            mem = o[:, :M, :].copy()
            outs.append(o[:, M:, :])
        return jnp.concatenate(outs, axis=1)

    def _B_ref(x, w_r, w_gate, w_up, w_down):
        B, S, D = x.shape
        C = 1
        r = x @ w_r
        idx = jnp.argsort(-r, axis=-1)[:, :C]
        idx_e = jnp.repeat(idx.reshape(B, C, 1), D, axis=2)
        x_sel = jnp.take_along_axis(x, idx_e, axis=1)
        g = _silu(x_sel @ w_gate)
        u = x_sel @ w_up
        y = g * u @ w_down
        r_sel = _sigmoid(jnp.take_along_axis(r, idx, axis=1))
        y = y * r_sel.reshape(B, C, 1)
        b_off = (jnp.arange(B) * S).reshape(B, 1)
        flat_idx = (idx + b_off).reshape(B * C)
        zero = (x * 0.0).reshape(B * S, D)
        upd = _scatter_add(zero, flat_idx, y.reshape(B * C, D), axis=0)
        return x + upd.reshape(B, S, D)
    x = A_x
    mod = (_silu(c) @ w_mod).reshape(c.shape[0], 6, 1, -1)
    sa, ca, ga, sb, cb, gb = (mod[:, 0].copy(), mod[:, 1].copy(), mod[:, 2].copy(), mod[:, 3].copy(), mod[:, 4].copy(), mod[:, 5].copy())
    h = _layernorm(x, axis=-1) * (1 + ca) + sa
    x = x + ga * _A_ref(h, A_mem0, A_Wq, A_Wk, A_Wv, A_Wo, A_seg_len)
    h = _layernorm(x, axis=-1) * (1 + cb) + sb
    x = x + gb * _B_ref(h, B_w_r, B_w_gate, B_w_up, B_w_down)
    return x
```

```python
import functools
import jax
import jax.numpy as jnp
from jax import lax
import jax.experimental.pallas as pl
import jax.experimental.pallas.tpu as pltpu

D = 448
DP = 512
DM = 384
H = 16
E = 256
M = 8
SEG = 32
S = 2048
NSEG = S // SEG
NPAIR = H // 2
CH = 2 * D
NCH = 2 * NPAIR
RIDE = 24
F = 1792
EPS = 1e-5
BF = jnp.bfloat16
F32 = jnp.float32


def _dot(a, b):
    return jnp.dot(a, b, preferred_element_type=F32)


def _dot_nt(a, b):
    return lax.dot_general(a, b, (((1,), (1,)), ((), ())), preferred_element_type=F32)


def _rb(x):
    return x.astype(BF).astype(F32)


def _ln_dup(x):
    m = jnp.sum(x[:, :D], axis=-1, keepdims=True) * (1.0 / D)
    xc = x - m
    xs = xc[:, :D]
    v = jnp.sum(xs * xs, axis=-1, keepdims=True) * (1.0 / D)
    return xc * lax.rsqrt(v + EPS)


def _dup(x):
    return jnp.concatenate([x, x[:, DM:D]], axis=1)


def _pack_block(blk, lo_mask):
    sh = blk[:, 2 * DM:]
    top = jnp.concatenate([blk[:, :DM], jnp.where(lo_mask, sh, 0.0)], axis=1)
    bot = jnp.concatenate([blk[:, DM:2 * DM], jnp.where(lo_mask, 0.0, sh)], axis=1)
    return jnp.concatenate([top, bot], axis=0).astype(BF)


def _group_allreduce(x, op, lane):
    for sh in (1, 2, 4):
        up = pltpu.roll(x, sh, 1)
        dn = pltpu.roll(x, 128 - sh, 1)
        x = op(x, jnp.where((lane & sh) != 0, up, dn))
    return x


def _kernel(xt_hbm, mem0_ref, wq_hbm, wk_hbm, wv_hbm, wo_hbm, wr_ref, wg_hbm, wu_hbm, wd_hbm,
            c_ref, wmod_hbm, out_hbm,
            xts, wqs, wks, wvs, wos, wgs, wus, wds, wms,
            wcat, hbuf, xbuf, hx, zum, zur, zue, membuf, obuf, x2buf, orow, modbuf, best, ost,
            sa_sems, sb_sems, x_sems, m_sems, osems):
    lane8 = lax.broadcasted_iota(jnp.int32, (8, 128), 1)
    lo_mask = lane8 < 64

    wk32 = wk_hbm.bitcast(jnp.uint32)
    wq32 = wq_hbm.bitcast(jnp.uint32)
    wv32 = wv_hbm.bitcast(jnp.uint32)

    def cp_a(p):
        return [pltpu.make_async_copy(wk32.at[:, p, :], wks.at[p], sa_sems.at[p]),
                pltpu.make_async_copy(wq32.at[:, p, :], wqs.at[p], sb_sems.at[p])]

    def cp_b(p):
        return [pltpu.make_async_copy(wv32.at[:, p, :], wvs.at[p], sa_sems.at[NPAIR + p]),
                pltpu.make_async_copy(wo_hbm.at[p], wos.at[p], sb_sems.at[NPAIR + p])]

    def cp_x(k):
        return pltpu.make_async_copy(xt_hbm.at[:, pl.ds(k * 256, 256)], xts.at[k], x_sems.at[k])

    cp_wm0 = pltpu.make_async_copy(wmod_hbm.at[:, pl.ds(0, CH)], wms.at[:, pl.ds(0, CH)], m_sems.at[0])
    cp_wm1 = pltpu.make_async_copy(wmod_hbm.at[:, pl.ds(CH, 2 * CH)], wms.at[:, pl.ds(CH, 2 * CH)], m_sems.at[1])
    cps_mlp = [pltpu.make_async_copy(s_, d_, m_sems.at[2 + i])
               for i, (s_, d_) in enumerate(((wg_hbm, wgs), (wu_hbm, wus), (wd_hbm, wds)))]

    for p in range(NPAIR):
        for cp in cp_a(p):
            cp.start()
    cp_wm0.start()
    for p in range(NPAIR):
        cp_x(p).start()
        for cp in cp_b(p):
            cp.start()
    cp_wm1.start()
    for cp in cps_mlp:
        cp.start()

    c = c_ref[...].astype(F32)
    sc = jnp.broadcast_to((c * jax.nn.sigmoid(c)).astype(BF), (8, D))
    membuf[...] = _dup(mem0_ref[...].astype(F32))
    obuf[...] = jnp.zeros((SEG, DP), F32)
    orow[0, pl.ds(0, 128), :] = jnp.zeros((128, 256), F32)
    best[0] = jnp.full((SEG, 1), -jnp.inf, F32)
    best[1] = jnp.zeros((SEG, 1), F32)

    def ln_pair(k):
        for half in range(2):
            r0 = pl.multiple_of(k * 256 + half * 128, 128)
            xt = xts[k, :, half * 128:(half + 1) * 128].astype(F32)
            x = jnp.concatenate([xt, xt[DM:]], axis=0).T
            xbuf[pl.ds(r0, 128), :] = x
            h = _ln_dup(x) * _rb(1.0 + modbuf[1][0:1]) + modbuf[0][0:1]
            hbuf[pl.ds(r0, 128), :] = h
            hx[pl.ds(pl.multiple_of(k * 64 + half * 32, 32), 32), :] = jnp.concatenate(
                [h[j * SEG + RIDE:(j + 1) * SEG] for j in range(4)], axis=0).astype(BF)

    def head_pair(v):
        return (pltpu.bitcast(v << 16, F32).astype(BF),
                pltpu.bitcast(v & jnp.uint32(0xFFFF0000), F32).astype(BF))

    def fold(cidx, a0, a1, b0, b1, scale):
        wcat[cidx, :, 0:DM] = (_dot_nt(a0, b0[:DM]) * scale).astype(BF)
        wcat[cidx, :, DM:2 * DM] = (_dot_nt(a1, b1[:DM]) * scale).astype(BF)
        z = jnp.zeros((D - DM, E), BF)
        bd = jnp.concatenate([jnp.concatenate([b0[DM:], z], axis=1),
                              jnp.concatenate([z, b1[DM:]], axis=1)], axis=0)
        wcat[cidx, :, 2 * DM:] = (_dot_nt(jnp.concatenate([a0, a1], axis=1), bd) * scale).astype(BF)

    def fold_a(p):
        a0, a1 = head_pair(wks[p])
        b0, b1 = head_pair(wqs[p])
        fold(p, a0, a1, b0, b1, E ** -0.5)

    def fold_b(p):
        a0, a1 = head_pair(wvs[p])
        fold(NPAIR + p, a0, a1, wos[p, 0:D, :], wos[p, D:CH, :], 1.0)

    def p0(cidx):
        l0 = jnp.concatenate([hx[pl.ds(0, 64), :], hbuf[pl.ds(0, 32), :].astype(BF)], axis=0)
        y = _dot(l0[:, :D], wcat[cidx])
        for i in range(8):
            zue[i, cidx] = _pack_block(y[8 * i:8 * i + 8], lo_mask)
        for j in range(3):
            zur[0, j, cidx] = _pack_block(y[64 + 8 * j:64 + 8 * j + 8], lo_mask)

    def fa_body(p, carry):
        for cp in cp_a(p):
            cp.wait()
        fold_a(p)
        return carry
    lax.fori_loop(0, NPAIR, fa_body, 0)

    cp_wm0.wait()
    cp_x(0).wait()
    for cp in cp_b(0):
        cp.wait()
    mod = _rb(_dot(sc, wms[:, pl.ds(0, CH)]))
    for i in range(2):
        modbuf[i] = _dup(mod[:, i * D:(i + 1) * D])
    fold_b(0)
    ln_pair(0)

    def fb_body(p, carry):
        cp_x(p).wait()
        for cp in cp_b(p):
            cp.wait()
        p0(2 * p - 2)
        p0(2 * p - 1)
        fold_b(p)
        ln_pair(p)
        return carry
    lax.fori_loop(1, NPAIR, fb_body, 0)

    cp_wm1.wait()
    p0(NCH - 2)
    mod = _rb(_dot(sc, wms[:, pl.ds(CH, 2 * CH)]))
    for i in range(4):
        modbuf[2 + i] = _dup(mod[:, i * D:(i + 1) * D])
    p0(NCH - 1)

    ga = modbuf[2][0:1]
    sb = modbuf[3][0:1]
    cb1 = _rb(1.0 + modbuf[4][0:1])
    gb = modbuf[5][0:1]
    wr = wr_ref[...].astype(F32)

    L = M + SEG
    row = lax.broadcasted_iota(jnp.int32, (L, 5 * 128), 0)
    col = lax.broadcasted_iota(jnp.int32, (L, 5 * 128), 1)
    kidx = (col // 128) * 8 + (col % 8)
    amask = jnp.logical_or(row < M, row >= kidx)
    lane40 = lax.broadcasted_iota(jnp.int32, (L, 128), 1)

    def epilogue(seg):
        r0 = pl.multiple_of(jnp.maximum(seg, 0) * SEG, SEG)
        attn = _rb(obuf[...])
        x = xbuf[pl.ds(r0, SEG), :]
        x2 = _rb(x + _rb(ga * attn))
        h2 = _rb(_ln_dup(x2) * cb1 + sb)
        r = _rb(jnp.sum(h2[:, :D] * wr, axis=-1, keepdims=True))
        x2buf[pl.ds(r0, SEG), :] = x2
        res = x2 + _rb(gb * h2)
        orow[0, pl.ds(r0, SEG), :] = res[:, :256]
        orow[1, pl.ds(r0, SEG), :] = res[:, 256:]
        bv = best[0]
        upd = jnp.logical_and(r > bv, seg >= 0)
        best[0] = jnp.where(upd, r, bv)
        best[1] = jnp.where(upd, seg.astype(F32), best[1])

    def out_copy(b, slot):
        return pltpu.make_async_copy(ost.at[slot, pl.ds(0, D), :],
                                     out_hbm.at[:, pl.ds(pl.multiple_of(b * 128, 128), 128)], osems.at[slot])

    def trans_half(b, half, slot):
        r0 = pl.multiple_of(b * 128, 128)
        ost[slot, pl.ds(pl.multiple_of(half * 256, 256), 256), :] = orow[half, pl.ds(r0, 128), :].T.astype(BF)

    def trans_step(i):
        t = jnp.maximum(i - 3, 0)
        trans_half(t // 2, t % 2, t // 2)

    def trans_dma(i):
        t = i - 3

        @pl.when(jnp.logical_and(t >= 0, t % 2 == 1))
        def _():
            out_copy(t // 2, t // 2).start()

    def extra(s, half):
        b = s // 8 + 1
        cidx = (s % 8) * 2 + half
        y = _dot(hx[pl.ds(pl.multiple_of(b * 64, 64), 64), :][:, :D], wcat[cidx])
        for i in range(8):
            zue[b * 8 + i, cidx] = _pack_block(y[8 * i:8 * i + 8], lo_mask)

    def step(s, slot, with_extra):
        mem = membuf[...]
        nxt = jnp.minimum(s + 1, NSEG - 1)
        ride = hbuf[pl.ds(pl.multiple_of(nxt * SEG, SEG), RIDE), :]
        lhs = jnp.concatenate([mem, ride], axis=0)[:, :D].astype(BF)
        q = jnp.concatenate([mem, hbuf[pl.ds(pl.multiple_of(s * SEG, SEG), SEG), :]], axis=0).astype(BF)

        def do_chunk(cidx):
            y = _dot(lhs, wcat[cidx])
            zum[cidx] = _pack_block(y[0:8], lo_mask)
            for j in range(3):
                zur[1 - slot, j, cidx] = _pack_block(y[8 * j + 8:8 * j + 16], lo_mask)

        epilogue(s - 1)

        for cidx in range(NPAIR):
            do_chunk(cidx)
        s_r = _dot_nt(q, zur[slot, :, 0:NPAIR].reshape(3 * 128, DP))
        s_e = _dot_nt(q, zue[s, 0:NPAIR].reshape(128, DP))
        s_m = _dot_nt(q, zum[0:NPAIR].reshape(128, DP))
        for cidx in range(NPAIR, NPAIR + 6):
            do_chunk(cidx)
        sc_ = jnp.concatenate([s_m, s_r, s_e], axis=1)
        sc_ = jnp.where(amask, sc_, -1e9)
        tiles = [sc_[:, j * 128:(j + 1) * 128] for j in range(5)]
        mx = functools.reduce(jnp.maximum, tiles)
        mx = _group_allreduce(mx, jnp.maximum, lane40)
        es = [jnp.exp(t - mx) for t in tiles]
        sm = functools.reduce(jnp.add, es)
        sm = _group_allreduce(sm, jnp.add, lane40)
        inv = 1.0 / sm
        ps = [(e * inv).astype(BF) for e in es]
        for cidx in range(NPAIR + 6, NCH):
            do_chunk(cidx)
        o = _dot(jnp.concatenate(ps[1:4], axis=1), zur[slot, :, NPAIR:].reshape(3 * 128, DP))
        o = o + _dot(ps[4], zue[s, NPAIR:].reshape(128, DP))
        if with_extra:
            extra(s, 0)
        o = o + _dot(ps[0], zum[NPAIR:].reshape(128, DP))
        o3 = o[:, DM:]
        o3 = o3 + pltpu.roll(o3, 64, 1)
        o = jnp.concatenate([o[:, :DM], o3], axis=1)
        membuf[...] = o[0:M]
        obuf[...] = o[M:]
        if with_extra:
            extra(s, 1)

    def body_a(i, carry):
        trans_step(i)
        step(2 * i, 0, True)
        step(2 * i + 1, 1, True)
        trans_dma(i)
        return carry
    lax.fori_loop(0, 28, body_a, 0)

    def body_b(i, carry):
        trans_step(i)
        step(2 * i, 0, False)
        step(2 * i + 1, 1, False)
        trans_dma(i)
        return carry
    lax.fori_loop(28, 32, body_b, 0)
    epilogue(jnp.int32(NSEG - 1))

    trans_half(14, 1, 14)
    out_copy(14, 14).start()
    trans_half(15, 0, 15)
    trans_half(15, 1, 15)
    out_copy(15, 15).start()

    for cp in cps_mlp:
        cp.wait()
    bv = best[0]
    rmax = jnp.max(bv, axis=0, keepdims=True)
    tok = best[1] * SEG + lax.broadcasted_iota(jnp.int32, (SEG, 1), 0).astype(F32)
    idx_f = jnp.min(jnp.where(bv == rmax, tok, float(S)), axis=0, keepdims=True)
    idx = jnp.clip(idx_f[0, 0].astype(jnp.int32), 0, S - 1)
    blk = pl.multiple_of((idx // 16) * 16, 16)
    x2 = x2buf[pl.ds(blk, 16), :]
    h2 = _rb(_ln_dup(x2) * cb1 + sb)
    h2b = h2[:, :D].astype(BF)
    g = _rb(_dot(h2b, wgs[...]))
    g = _rb(g * jax.nn.sigmoid(g))
    u = _rb(_dot(h2b, wus[...]))
    y = _rb(_dot_nt((g * u).astype(BF), wds[...]))
    y = _dup(_rb(y * _rb(jax.nn.sigmoid(rmax))))
    sel = lax.broadcasted_iota(jnp.int32, (16, DP), 0) == (idx - blk)
    bo = _rb(h2 + jnp.where(sel, y, 0.0))
    res = x2 + _rb(gb * bo)
    orow[0, pl.ds(blk, 16), :] = res[:, :256]
    orow[1, pl.ds(blk, 16), :] = res[:, 256:]
    fb = idx // 128
    trans_half(fb, 0, 16)
    trans_half(fb, 1, 16)
    for b_ in range(16):
        out_copy(b_, b_).wait()
    fix = out_copy(fb, 16)
    fix.start()
    fix.wait()


@jax.jit
def pallas_adaLN_cond__memory_aug_recurrent_mem_tr__moe_arch_mod__prompt_kernel(A_x, A_mem0, A_Wq, A_Wk, A_Wv, A_Wo, A_seg_len, B_x, B_w_r, B_w_gate, B_w_up, B_w_down, c, w_mod):
    vm = pl.BlockSpec(memory_space=pltpu.VMEM)
    hbm = pl.BlockSpec(memory_space=pltpu.HBM)
    out = pl.pallas_call(
        _kernel,
        out_shape=jax.ShapeDtypeStruct((D, S), BF),
        in_specs=[hbm, vm, hbm, hbm, hbm, hbm, vm, hbm, hbm, hbm, vm, hbm],
        out_specs=hbm,
        scratch_shapes=[
            pltpu.VMEM((8, D, 256), BF),
            pltpu.VMEM((NPAIR, D, E), jnp.uint32),
            pltpu.VMEM((NPAIR, D, E), jnp.uint32),
            pltpu.VMEM((NPAIR, D, E), jnp.uint32),
            pltpu.VMEM((NPAIR, CH, E), BF),
            pltpu.VMEM((D, F), BF),
            pltpu.VMEM((D, F), BF),
            pltpu.VMEM((D, F), BF),
            pltpu.VMEM((D, 6 * D), BF),
            pltpu.VMEM((NCH, D, CH), BF),
            pltpu.VMEM((S, DP), F32),
            pltpu.VMEM((S, DP), F32),
            pltpu.VMEM((NSEG * 8, DP), BF),
            pltpu.VMEM((NCH, 16, DP), BF),
            pltpu.VMEM((2, 3, NCH, 16, DP), BF),
            pltpu.VMEM((NSEG, NCH, 16, DP), BF),
            pltpu.VMEM((M, DP), F32),
            pltpu.VMEM((SEG, DP), F32),
            pltpu.VMEM((S, DP), F32),
            pltpu.VMEM((2, S, 256), F32),
            pltpu.VMEM((6, 8, DP), F32),
            pltpu.VMEM((2, SEG, 1), F32),
            pltpu.VMEM((17, DP, 128), BF),
            pltpu.SemaphoreType.DMA((NCH,)),
            pltpu.SemaphoreType.DMA((NCH,)),
            pltpu.SemaphoreType.DMA((8,)),
            pltpu.SemaphoreType.DMA((5,)),
            pltpu.SemaphoreType.DMA((17,)),
        ],
        compiler_params=pltpu.CompilerParams(vmem_limit_bytes=110 * 1024 * 1024),
    )(A_x.reshape(S, D).T, A_mem0.reshape(M, D), A_Wq, A_Wk, A_Wv,
      jnp.transpose(A_Wo, (0, 2, 1)).reshape(NPAIR, CH, E), B_w_r.reshape(1, D),
      B_w_gate, B_w_up, B_w_down.T, c, w_mod)
    return out.T.reshape(1, S, D)
```

```python
import functools
import jax
import jax.numpy as jnp
from jax import lax
import jax.experimental.pallas as pl
import jax.experimental.pallas.tpu as pltpu

D = 448
DP = 512
DM = 384
H = 16
E = 256
M = 8
SEG = 32
S = 2048
NSEG = S // SEG
NPAIR = H // 2
CH = 2 * D
NCH = 2 * NPAIR
RIDE = 24
F = 1792
NPRE = 2
EPS = 1e-5
BF = jnp.bfloat16
F32 = jnp.float32


def _dot(a, b):
    return jnp.dot(a, b, preferred_element_type=F32)


def _dot_nt(a, b):
    return lax.dot_general(a, b, (((1,), (1,)), ((), ())), preferred_element_type=F32)


def _st(x):
    return pltpu.bitcast(x, jnp.uint32)


def _ld(x):
    return pltpu.bitcast(x, BF)


def _rb(x):
    return x.astype(BF).astype(F32)


def _ln_dup(x):
    m = jnp.sum(x[:, :D], axis=-1, keepdims=True) * (1.0 / D)
    xc = x - m
    xs = xc[:, :D]
    v = jnp.sum(xs * xs, axis=-1, keepdims=True) * (1.0 / D)
    return xc * lax.rsqrt(v + EPS)


def _dup(x):
    return jnp.concatenate([x, x[:, DM:D]], axis=1)


def _pack_block(blk, lo_mask):
    sh = blk[:, 2 * DM:]
    top = jnp.concatenate([blk[:, :DM], jnp.where(lo_mask, sh, 0.0)], axis=1)
    bot = jnp.concatenate([blk[:, DM:2 * DM], jnp.where(lo_mask, 0.0, sh)], axis=1)
    return _st(jnp.concatenate([top, bot], axis=0).astype(BF))


def _group_allreduce(x, op, lane):
    for sh in (1, 2, 4):
        up = pltpu.roll(x, sh, 1)
        dn = pltpu.roll(x, 128 - sh, 1)
        x = op(x, jnp.where((lane & sh) != 0, up, dn))
    return x


def _kernel(xt_hbm, mem0_hbm, wq_hbm, wk_hbm, wv_hbm, wo_hbm, wr_hbm, wg_hbm, wu_hbm, wd_hbm,
            c_hbm, wmod_hbm, out_hbm,
            xts, wqs, wks, wvs, wos, wgs, wus, wds, wms,
            wcat, hbuf, xbuf, hx, zur, zue, membuf, obuf, x2buf, orow, modbuf, ost, spec_y,
            mem0_ref, wr_ref, c_ref, spec_idx,
            c_sems, m_sems, osems):
    lane8 = lax.broadcasted_iota(jnp.int32, (8, 128), 1)
    lo_mask = lane8 < 64

    wk32 = wk_hbm.bitcast(jnp.uint32)
    wq32 = wq_hbm.bitcast(jnp.uint32)
    wv32 = wv_hbm.bitcast(jnp.uint32)

    def cp_a(p):
        return [pltpu.make_async_copy(wk32.at[:, p, :], wks.at[p], c_sems.at[p]),
                pltpu.make_async_copy(wq32.at[:, p, :], wqs.at[p], c_sems.at[p])]

    def cp_b(p):
        return [pltpu.make_async_copy(wv32.at[:, p, :], wvs.at[p], c_sems.at[NPAIR + p]),
                pltpu.make_async_copy(wo_hbm.at[p], wos.at[p], c_sems.at[NPAIR + p])]

    def cp_x(k):
        return pltpu.make_async_copy(xt_hbm.at[:, pl.ds(k * 256, 256)], xts.at[k], c_sems.at[NPAIR + k])

    cp_wm0 = pltpu.make_async_copy(wmod_hbm.at[:, pl.ds(0, CH)], wms.at[:, pl.ds(0, CH)], c_sems.at[NPAIR])
    cp_wm1 = pltpu.make_async_copy(wmod_hbm.at[:, pl.ds(CH, 2 * CH)], wms.at[:, pl.ds(CH, 2 * CH)], m_sems.at[0])
    cps_mlp = [pltpu.make_async_copy(s_, d_, m_sems.at[1])
               for s_, d_ in ((wg_hbm, wgs), (wu_hbm, wus), (wd_hbm, wds))]

    for p in range(NPAIR):
        for cp in cp_a(p):
            cp.start()
    cps_small = [pltpu.make_async_copy(s_, d_, c_sems.at[NPAIR])
                 for s_, d_ in ((mem0_hbm, mem0_ref), (wr_hbm, wr_ref), (c_hbm, c_ref))]
    for cp in cps_small:
        cp.start()
    cp_wm0.start()
    for p in range(NPAIR):
        cp_x(p).start()
        for cp in cp_b(p):
            cp.start()
    cp_wm1.start()

    obuf[...] = jnp.zeros((SEG, DP), F32)
    orow[0, pl.ds(0, 128), :] = jnp.zeros((128, 256), F32)
    orow[1, pl.ds(0, 128), :] = jnp.zeros((128, 256), F32)
    hbuf[S:S + SEG, 0:1] = jnp.full((SEG, 1), -jnp.inf, F32)
    hbuf[S + SEG:S + 2 * SEG, 0:1] = jnp.zeros((SEG, 1), F32)

    def ln_pair(k):
        for half in range(2):
            r0 = pl.multiple_of(k * 256 + half * 128, 128)
            xt = xts[k, :, half * 128:(half + 1) * 128].astype(F32)
            x = jnp.concatenate([xt, xt[DM:]], axis=0).T
            xbuf[pl.ds(r0, 128), :] = x
            h = _ln_dup(x) * _rb(1.0 + modbuf[1][0:1]) + modbuf[0][0:1]
            hbuf[pl.ds(r0, 128), :] = h
            hx[pl.ds(pl.multiple_of(k * 32 + half * 16, 16), 16), :] = _st(jnp.concatenate(
                [h[j * SEG + RIDE:(j + 1) * SEG] for j in range(4)], axis=0).astype(BF))

    def head_pair(v):
        return (pltpu.bitcast(v << 16, F32).astype(BF),
                pltpu.bitcast(v & jnp.uint32(0xFFFF0000), F32).astype(BF))

    def fold(cidx, a0, a1, b0, b1, scale):
        a0p = jnp.concatenate([a0, a0[DM:]], axis=0)
        a1p = jnp.concatenate([a1, a1[DM:]], axis=0)
        sh_t = jnp.concatenate([_dot_nt(b0[DM:], a0p), _dot_nt(b1[DM:], a1p)], axis=0)
        wcat[cidx, :, 2 * DM:] = _st((sh_t.T[:D] * scale).astype(BF))
        wcat[cidx, :, 0:DM] = _st((_dot_nt(a0, b0[:DM]) * scale).astype(BF))
        wcat[cidx, :, DM:2 * DM] = _st((_dot_nt(a1, b1[:DM]) * scale).astype(BF))

    def fold_a(p):
        a0, a1 = head_pair(wks[p])
        b0, b1 = head_pair(wqs[p])
        fold(p, a0, a1, b0, b1, E ** -0.5)

    def fold_b(p):
        a0, a1 = head_pair(wvs[p])
        fold(NPAIR + p, a0, a1, wos[p, 0:D, :], wos[p, D:CH, :], 1.0)

    def p0(cidx):
        y = _dot(_ld(hx[pl.ds(0, 32), :])[:, :D], _ld(wcat[cidx]))
        for i in range(8):
            zue[i, cidx] = _pack_block(y[8 * i:8 * i + 8], lo_mask)

    def fa_body(p, carry):
        for cp in cp_a(p):
            cp.wait()
        fold_a(p)
        return carry
    lax.fori_loop(0, NPAIR, fa_body, 0)

    cp_wm0.wait()
    cp_x(0).wait()
    for cp in cp_b(0) + cps_small:
        cp.wait()
    c = c_ref[...].astype(F32)
    sc = jnp.broadcast_to((c * jax.nn.sigmoid(c)).astype(BF), (8, D))
    membuf[...] = _dup(mem0_ref[...].astype(F32))
    mod = _rb(_dot(sc, wms[:, pl.ds(0, CH)]))
    for i in range(2):
        modbuf[i] = _dup(mod[:, i * D:(i + 1) * D])
    fold_b(0)
    ln_pair(0)

    def fb_body(p, carry):
        cp_x(p).wait()
        for cp in cp_b(p):
            cp.wait()
        p0(2 * p - 2)
        p0(2 * p - 1)
        fold_b(p)
        ln_pair(p)
        return carry
    lax.fori_loop(1, NPAIR, fb_body, 0)

    cp_wm1.wait()
    for cp in cps_mlp:
        cp.start()
    p0(NCH - 2)
    mod = _rb(_dot(sc, wms[:, pl.ds(CH, 2 * CH)]))
    for i in range(4):
        modbuf[2 + i] = _dup(mod[:, i * D:(i + 1) * D])
    p0(NCH - 1)

    ga = modbuf[2][0:1]
    sb = modbuf[3][0:1]
    cb1 = _rb(1.0 + modbuf[4][0:1])
    gb = modbuf[5][0:1]
    wr = wr_ref[...].astype(F32).reshape(1, D)

    L = M + SEG
    diag = lax.broadcasted_iota(jnp.int32, (8, 128), 0) >= (lane8 % 8)
    lane40 = lax.broadcasted_iota(jnp.int32, (L, 128), 1)

    def epilogue(seg):
        r0 = pl.multiple_of(jnp.maximum(seg, 0) * SEG, SEG)
        attn = _rb(obuf[...])
        x = xbuf[pl.ds(r0, SEG), :]
        x2 = _rb(x + _rb(ga * attn))
        h2 = _rb(_ln_dup(x2) * cb1 + sb)
        r = _rb(jnp.sum(h2[:, :D] * wr, axis=-1, keepdims=True))
        x2buf[pl.ds(r0, SEG), :] = x2
        res = x2 + _rb(gb * h2)
        orow[0, pl.ds(r0, SEG), :] = res[:, :256]
        orow[1, pl.ds(r0, SEG), :] = res[:, 256:]
        bv = hbuf[S:S + SEG, 0:1]
        upd = jnp.logical_and(r > bv, seg >= 0)
        hbuf[S:S + SEG, 0:1] = jnp.where(upd, r, bv)
        hbuf[S + SEG:S + 2 * SEG, 0:1] = jnp.where(upd, seg.astype(F32), hbuf[S + SEG:S + 2 * SEG, 0:1])

    def out_copy(b, slot):
        return pltpu.make_async_copy(ost.at[slot, pl.ds(0, D), :],
                                     out_hbm.at[:, pl.ds(pl.multiple_of(b * 128, 128), 128)], osems.at[0])

    def trans_half(b, half, slot):
        r0 = pl.multiple_of(b * 128, 128)
        ost[slot, half * 256:(half + 1) * 256, :] = orow[half, pl.ds(r0, 128), :].T.astype(BF)

    def trans_block(b, slot):
        trans_half(b, 0, slot)
        trans_half(b, 1, slot)

    def extra_parts(s, half):
        b = s // 8 + 1
        cidx = (s % 8) * 2 + half
        lx = _ld(hx[pl.ds(pl.multiple_of(b * 32, 32), 32), :])[:, :D]

        def tile(t):
            return _dot(lx, _ld(wcat[cidx, :, t * 128:(t + 1) * 128]))

        def finish(ts):
            y = jnp.concatenate(ts, axis=1)
            for i in range(8):
                zue[b * 8 + i, cidx] = _pack_block(y[8 * i:8 * i + 8], lo_mask)
        return tile, finish

    def step(s, with_extra, fill1=None, fill2=None):
        mem = membuf[...]
        hs = hbuf[pl.ds(pl.multiple_of(s * SEG, SEG), RIDE), :]
        lhs = jnp.concatenate([mem, hs], axis=0)[:, :D].astype(BF)
        epilogue(s - 1)
        hs3 = hbuf[pl.ds(pl.multiple_of(s * SEG + RIDE, 8), 8), :]
        q = jnp.concatenate([mem, hs3, hs[16:24], hs[8:16], hs[0:8]], axis=0).astype(BF)
        nrow = (40, 40, 32, 24, 16)

        def do_chunk(cidx):
            y = _dot(lhs, _ld(wcat[cidx]))
            for j in range(4):
                zur[j, cidx] = _pack_block(y[8 * j:8 * j + 8], lo_mask)

        def kv_tile(j, lo):
            z = zue[s, lo:lo + NPAIR] if j == 4 else zur[j, lo:lo + NPAIR]
            return _ld(z.reshape(64, DP))

        def s_tile(j):
            n16 = -(-nrow[j] // 16) * 16
            return _dot_nt(q[:min(n16, L)], kv_tile(j, 0))

        for cidx in range(NPAIR + 1):
            do_chunk(cidx)
        tiles = [None] * 5
        if with_extra:
            etile0, efin0 = extra_parts(s, 0)
            ets0 = []
            for n, j in enumerate((0, 4, 1, 3, 2)):
                ets0.append(etile0(n))
                tiles[j] = s_tile(j)
        else:
            for j in (4, 0, 1, 2, 3):
                tiles[j] = s_tile(j)
        for cidx in range(NPAIR + 1, NPAIR + 7):
            do_chunk(cidx)
        blocks = []
        for j in range(5):
            nb = nrow[j] // 8
            bl = [tiles[j][8 * rb:8 * rb + 8] for rb in range(nb)]
            if j >= 1:
                bl[-1] = jnp.where(diag, bl[-1], -1e9)
            blocks.append(bl)
        per_rb = lambda xs, rb: [xs[j][rb] for j in range(5) if rb < len(xs[j])]
        mx = jnp.concatenate([functools.reduce(jnp.maximum, per_rb(blocks, rb)) for rb in range(5)], axis=0)
        mx = _group_allreduce(mx, jnp.maximum, lane40)
        es = [[jnp.exp(b_ - mx[8 * rb:8 * rb + 8]) for rb, b_ in enumerate(bl)] for bl in blocks]
        sm = jnp.concatenate([functools.reduce(jnp.add, per_rb(es, rb)) for rb in range(5)], axis=0)
        sm = _group_allreduce(sm, jnp.add, lane40)
        inv = 1.0 / sm
        ps = [(jnp.concatenate(es[j], axis=0) * inv[:nrow[j]]).astype(BF) for j in range(5)]
        for cidx in range(NPAIR + 7, NCH):
            do_chunk(cidx)
        os_ = [None] * 5
        os_[4] = _dot(ps[4], kv_tile(4, NPAIR))
        if with_extra:
            ets0 += [etile0(5), etile0(6)]
            efin0(ets0)
            etile, efin = extra_parts(s, 1)
            ets = [etile(n) for n in range(NPRE)]
        if fill1 is not None:
            fill1()
        for j in (0, 1, 2, 3):
            os_[j] = _dot(ps[j], kv_tile(j, NPAIR))
        ob = [[os_[j][8 * rb:8 * rb + 8] for rb in range(nrow[j] // 8)] for j in range(5)]
        o = jnp.concatenate([functools.reduce(jnp.add, per_rb(ob, rb)) for rb in (0, 4, 3, 2, 1)], axis=0)
        o3 = o[:, DM:]
        o3 = o3 + pltpu.roll(o3, 64, 1)
        o = jnp.concatenate([o[:, :DM], o3], axis=1)
        membuf[...] = o[0:M]
        obuf[...] = o[M:]
        if with_extra:
            ets += [etile(n) for n in range(NPRE, 7)]
            efin(ets)
        if fill2 is not None:
            fill2()

    def argmax_token():
        bv = hbuf[S:S + SEG, 0:1]
        rmax = jnp.max(bv, axis=0, keepdims=True)
        tok = hbuf[S + SEG:S + 2 * SEG, 0:1] * SEG + lax.broadcasted_iota(jnp.int32, (SEG, 1), 0).astype(F32)
        idx_f = jnp.min(jnp.where(bv == rmax, tok, float(S)), axis=0, keepdims=True)
        return jnp.clip(idx_f[0, 0].astype(jnp.int32), 0, S - 1), rmax

    def mlp_stages(idx, half):
        blk = pl.multiple_of((idx // 16) * 16, 16)
        h2b = _rb(_ln_dup(x2buf[pl.ds(blk, 16), :]) * cb1 + sb)[:, :D].astype(BF)
        st = {}
        cuts = (0, 512, CH)

        def cols(k):
            return pl.ds(pl.multiple_of(half * CH + cuts[k], 128), cuts[k + 1] - cuts[k])

        def gu(name, w, k):
            def f():
                st[name, k] = _rb(_dot(h2b, w[:, cols(k)]))
            return f

        def dn(n):
            def f():
                if n == 0:
                    g = jnp.concatenate([st['g', 0], st['g', 1]], axis=1)
                    u = jnp.concatenate([st['u', 0], st['u', 1]], axis=1)
                    st['a'] = (_rb(g * jax.nn.sigmoid(g)) * u).astype(BF)
                hc = pl.ds(pl.multiple_of(half * CH, 128), CH)
                if n < 3:
                    wl = wds[n * 128:(n + 1) * 128, hc]
                else:
                    wl = wds[DM:D, hc]
                    wl = jnp.concatenate([wl, wl], axis=0)
                spec_y[:, n * 128:(n + 1) * 128] += _dot_nt(st['a'], wl)
            return f
        return [gu('g', wgs, 0), gu('g', wgs, 1), gu('u', wus, 0), gu('u', wus, 1), dn(0), dn(1), dn(2), dn(3)]

    def body(j, with_extra, dma=True):
        if with_extra:
            fl = [None] * 8
        else:
            fl = mlp_stages(spec_idx[0], j - 14)
        bprev = jnp.maximum(j - 1, 0)
        step(4 * j, with_extra, fl[0], fl[1])
        if not with_extra:
            trans_block(bprev, bprev)
        step(4 * j + 1, with_extra, fl[2], fl[3])
        step(4 * j + 2, with_extra, fl[4], fl[5])
        step(4 * j + 3, with_extra, fl[6], fl[7])
        if with_extra:
            trans_block(bprev, bprev)

        if dma:
            out_copy(bprev, bprev).start()

    def body_a(j, carry):
        body(2 * j, True, dma=False)
        body(2 * j + 1, True, dma=False)

        @pl.when(j >= 1)
        def _():
            out_copy(2 * j - 1, 2 * j - 1).start()
        out_copy(2 * j, 2 * j).start()
        return carry
    lax.fori_loop(0, 7, body_a, 0)

    for cp in cps_mlp:
        cp.wait()
    spec_idx[0] = jnp.minimum(argmax_token()[0], 55 * SEG - 1)
    spec_y[...] = jnp.zeros((16, DP), F32)

    def body_b(j, carry):
        body(j, False)
        return carry
    lax.fori_loop(14, 16, body_b, 0)
    epilogue(jnp.int32(NSEG - 1))
    trans_block(15, 15)
    out_copy(15, 15).start()

    idx, rmax = argmax_token()

    @pl.when(idx != spec_idx[0])
    def _():
        spec_y[...] = jnp.zeros((16, DP), F32)
        for half in range(2):
            for f in mlp_stages(idx, half):
                f()

    blk = pl.multiple_of((idx // 16) * 16, 16)
    x2 = x2buf[pl.ds(blk, 16), :]
    h2 = _rb(_ln_dup(x2) * cb1 + sb)
    y = _rb(_rb(spec_y[...]) * _rb(jax.nn.sigmoid(rmax)))
    sel = lax.broadcasted_iota(jnp.int32, (16, DP), 0) == (idx - blk)
    bo = _rb(h2 + jnp.where(sel, y, 0.0))
    res = x2 + _rb(gb * bo)
    orow[0, pl.ds(blk, 16), :] = res[:, :256]
    orow[1, pl.ds(blk, 16), :] = res[:, 256:]
    fb = idx // 128
    trans_block(fb, 16)
    for b_ in range(16):
        out_copy(b_, b_).wait()
    fix = out_copy(fb, 16)
    fix.start()
    fix.wait()


@jax.jit
def pallas_adaLN_cond__memory_aug_recurrent_mem_tr__moe_arch_mod__prompt_kernel(A_x, A_mem0, A_Wq, A_Wk, A_Wv, A_Wo, A_seg_len, B_x, B_w_r, B_w_gate, B_w_up, B_w_down, c, w_mod):
    hbm = pl.BlockSpec(memory_space=pltpu.HBM)
    out = pl.pallas_call(
        _kernel,
        out_shape=jax.ShapeDtypeStruct((D, S), BF),
        in_specs=[hbm] * 12,
        out_specs=hbm,
        scratch_shapes=[
            pltpu.VMEM((8, D, 256), BF),
            pltpu.VMEM((NPAIR, D, E), jnp.uint32),
            pltpu.VMEM((NPAIR, D, E), jnp.uint32),
            pltpu.VMEM((NPAIR, D, E), jnp.uint32),
            pltpu.VMEM((NPAIR, CH, E), BF),
            pltpu.VMEM((D, F), BF),
            pltpu.VMEM((D, F), BF),
            pltpu.VMEM((D, F), BF),
            pltpu.VMEM((D, 6 * D), BF),
            pltpu.VMEM((NCH, D // 2, CH), jnp.uint32),
            pltpu.VMEM((S + 2 * SEG, DP), F32),
            pltpu.VMEM((S, DP), F32),
            pltpu.VMEM((NSEG * 4, DP), jnp.uint32),
            pltpu.VMEM((4, NCH, 8, DP), jnp.uint32),
            pltpu.VMEM((NSEG, NCH, 8, DP), jnp.uint32),
            pltpu.VMEM((M, DP), F32),
            pltpu.VMEM((SEG, DP), F32),
            pltpu.VMEM((S, DP), F32),
            pltpu.VMEM((2, S, 256), F32),
            pltpu.VMEM((6, 8, DP), F32),
            pltpu.VMEM((17, DP, 128), BF),
            pltpu.VMEM((16, DP), F32),
            pltpu.VMEM((M, D), BF),
            pltpu.VMEM((D,), BF),
            pltpu.VMEM((1, D), BF),
            pltpu.SMEM((1,), jnp.int32),
            pltpu.SemaphoreType.DMA((NCH,)),
            pltpu.SemaphoreType.DMA((2,)),
            pltpu.SemaphoreType.DMA((1,)),
        ],
        compiler_params=pltpu.CompilerParams(vmem_limit_bytes=110 * 1024 * 1024),
    )(A_x.reshape(S, D).T, A_mem0.reshape(M, D), A_Wq, A_Wk, A_Wv,
      jnp.transpose(A_Wo, (0, 2, 1)).reshape(NPAIR, CH, E), B_w_r,
      B_w_gate, B_w_up, B_w_down.T, c, w_mod)
    return out.T.reshape(1, S, D)
```

```python
import functools
import jax
import jax.numpy as jnp
from jax import lax
import jax.experimental.pallas as pl
import jax.experimental.pallas.tpu as pltpu

D = 448
DP = 512
DM = 384
H = 16
E = 256
M = 8
SEG = 32
S = 2048
NSEG = S // SEG
NPAIR = H // 2
CH = 2 * D
NCH = 2 * NPAIR
RIDE = 24
F = 1792
NPRE = 2
EORD = (7, 0, 1, 2, 3, 4, 5, 6)
SORD = ((1, 'R'), (0, 4), (2, 3), (1, 2), (2, 0), (1, 1))
EPS = 1e-5
BF = jnp.bfloat16
F32 = jnp.float32


def _dot(a, b):
    return jnp.dot(a, b, preferred_element_type=F32)


def _dot_nt(a, b):
    return lax.dot_general(a, b, (((1,), (1,)), ((), ())), preferred_element_type=F32)


def _st(x):
    return pltpu.bitcast(x, jnp.uint32)


def _ld(x):
    return pltpu.bitcast(x, BF)


def _rb(x):
    return x.astype(BF).astype(F32)


def _ln_dup(x):
    m = jnp.sum(x[:, :D], axis=-1, keepdims=True) * (1.0 / D)
    xc = x - m
    xs = xc[:, :D]
    v = jnp.sum(xs * xs, axis=-1, keepdims=True) * (1.0 / D)
    return xc * lax.rsqrt(v + EPS)


def _dup(x):
    return jnp.concatenate([x, x[:, DM:D]], axis=1)


def _pack_block(blk, lo_mask):
    sh = blk[:, 2 * DM:]
    top = jnp.concatenate([blk[:, :DM], jnp.where(lo_mask, sh, 0.0)], axis=1)
    bot = jnp.concatenate([blk[:, DM:2 * DM], jnp.where(lo_mask, 0.0, sh)], axis=1)
    return _st(jnp.concatenate([top, bot], axis=0).astype(BF))


def _group_allreduce(x, op, lane):
    for sh in (1, 2, 4):
        up = pltpu.roll(x, sh, 1)
        dn = pltpu.roll(x, 128 - sh, 1)
        x = op(x, jnp.where((lane & sh) != 0, up, dn))
    return x


def _kernel(xt_hbm, mem0_hbm, wq_hbm, wk_hbm, wv_hbm, wo_hbm, wr_hbm, wg_hbm, wu_hbm, wd_hbm,
            c_hbm, wmod_hbm, out_hbm,
            xts, wqs, wks, wvs, wos, wgs, wus, wds, wms,
            wcat, wt2, wb2, t2e, hbuf, xbuf, hx, zur, zue, membuf, obuf, x2buf, orow, modbuf, ost, spec_y,
            mem0_ref, wr_ref, c_ref, spec_idx,
            c_sems, m_sems, osems):
    lane8 = lax.broadcasted_iota(jnp.int32, (8, 128), 1)
    lo_mask = lane8 < 64

    wk32 = wk_hbm.bitcast(jnp.uint32)
    wq32 = wq_hbm.bitcast(jnp.uint32)
    wv32 = wv_hbm.bitcast(jnp.uint32)

    def cp_a(p):
        return [pltpu.make_async_copy(wk32.at[:, p, :], wks.at[p], c_sems.at[p]),
                pltpu.make_async_copy(wq32.at[:, p, :], wqs.at[p], c_sems.at[p])]

    def cp_b(p):
        return [pltpu.make_async_copy(wv32.at[:, p, :], wvs.at[p], c_sems.at[NPAIR + p]),
                pltpu.make_async_copy(wo_hbm.at[p], wos.at[p], c_sems.at[NPAIR + p])]

    def cp_x(k):
        return pltpu.make_async_copy(xt_hbm.at[:, pl.ds(k * 256, 256)], xts.at[k], c_sems.at[NPAIR + k])

    cp_wm0 = pltpu.make_async_copy(wmod_hbm.at[:, pl.ds(0, CH)], wms.at[:, pl.ds(0, CH)], c_sems.at[NPAIR])
    cp_wm1 = pltpu.make_async_copy(wmod_hbm.at[:, pl.ds(CH, 2 * CH)], wms.at[:, pl.ds(CH, 2 * CH)], m_sems.at[0])
    cps_mlp = [pltpu.make_async_copy(s_, d_, m_sems.at[1])
               for s_, d_ in ((wg_hbm, wgs), (wu_hbm, wus), (wd_hbm, wds))]

    for p in range(NPAIR):
        for cp in cp_a(p):
            cp.start()
    cps_small = [pltpu.make_async_copy(s_, d_, c_sems.at[NPAIR])
                 for s_, d_ in ((mem0_hbm, mem0_ref), (wr_hbm, wr_ref), (c_hbm, c_ref))]
    for cp in cps_small:
        cp.start()
    cp_wm0.start()
    for p in range(NPAIR):
        cp_x(p).start()
        for cp in cp_b(p):
            cp.start()
    cp_wm1.start()

    obuf[...] = jnp.zeros((2, SEG, DP), F32)
    orow[0, pl.ds(0, 128), :] = jnp.zeros((128, 256), F32)
    orow[1, pl.ds(0, 128), :] = jnp.zeros((128, 256), F32)
    hbuf[S:S + SEG, 0:1] = jnp.full((SEG, 1), -jnp.inf, F32)
    hbuf[S + SEG:S + 2 * SEG, 0:1] = jnp.zeros((SEG, 1), F32)

    def ln_pair(k):
        for half in range(2):
            r0 = pl.multiple_of(k * 256 + half * 128, 128)
            xt = xts[k, :, half * 128:(half + 1) * 128].astype(F32)
            x = jnp.concatenate([xt, xt[DM:]], axis=0).T
            xbuf[pl.ds(r0, 128), :] = x
            h = _ln_dup(x) * _rb(1.0 + modbuf[1][0:1]) + modbuf[0][0:1]
            hbuf[pl.ds(r0, 128), :] = h
            hx[pl.ds(pl.multiple_of(k * 32 + half * 16, 16), 16), :] = _st(jnp.concatenate(
                [h[j * SEG + RIDE:(j + 1) * SEG] for j in range(4)], axis=0).astype(BF))

    def head_pair(v):
        return (pltpu.bitcast(v << 16, F32).astype(BF),
                pltpu.bitcast(v & jnp.uint32(0xFFFF0000), F32).astype(BF))

    def pad_rows(a):
        return jnp.concatenate([a, a[DM:]], axis=0)

    def fold_a(p):
        a0, a1 = head_pair(wks[p])
        b0, b1 = head_pair(wqs[p])
        scale = E ** -0.5
        sh_t = jnp.concatenate([_dot_nt(b0[DM:], a0[:DM]), _dot_nt(b1[DM:], a1[:DM])], axis=0)
        wcat[p, :, 2 * DM:] = _st((sh_t.T * scale).astype(BF))
        t2_t = jnp.concatenate([_dot_nt(a0[DM:], pad_rows(b0)), _dot_nt(a1[DM:], pad_rows(b1))], axis=0)
        wt2[p] = _st((t2_t.T[:D] * scale).astype(BF))
        wcat[p, :, 0:DM] = _st((_dot_nt(a0[:DM], b0[:DM]) * scale).astype(BF))
        wcat[p, :, DM:2 * DM] = _st((_dot_nt(a1[:DM], b1[:DM]) * scale).astype(BF))

    def fold_b(p):
        a0, a1 = head_pair(wvs[p])
        b0, b1 = wos[p, 0:D, :], wos[p, D:CH, :]
        cidx = NPAIR + p
        sh_t = jnp.concatenate([_dot_nt(b0[DM:], a0[:DM]), _dot_nt(b1[DM:], a1[:DM])], axis=0)
        wcat[cidx, :, 2 * DM:] = _st(sh_t.T.astype(BF))
        z = jnp.zeros((DP - D, E), BF)
        b2 = jnp.concatenate([_dot_nt(a0[DM:], jnp.concatenate([b0, z], axis=0)),
                              _dot_nt(a1[DM:], jnp.concatenate([b1, z], axis=0))], axis=0)
        wb2[p] = _st(b2.astype(BF))
        wcat[cidx, :, 0:DM] = _st(_dot_nt(a0[:DM], b0[:DM]).astype(BF))
        wcat[cidx, :, DM:2 * DM] = _st(_dot_nt(a1[:DM], b1[:DM]).astype(BF))

    def proj(lhs, cidx, lo=0, hi=CH):
        return _dot(lhs[:, :DM], _ld(wcat[cidx, :, lo:hi]))

    def p0(cidx, is_z):
        lx = _ld(hx[pl.ds(0, 32), :])
        y = proj(lx, cidx)
        for i in range(8):
            zue[i, cidx] = _pack_block(y[8 * i:8 * i + 8], lo_mask)
        if is_z:
            t2e[cidx, pl.ds(0, 64), :] = _dot(lx[:, :D], _ld(wt2[cidx]))

    def fa_body(p, carry):
        for cp in cp_a(p):
            cp.wait()
        fold_a(p)
        return carry
    lax.fori_loop(0, NPAIR, fa_body, 0)

    cp_wm0.wait()
    cp_x(0).wait()
    for cp in cp_b(0) + cps_small:
        cp.wait()
    c = c_ref[...].astype(F32)
    sc = jnp.broadcast_to((c * jax.nn.sigmoid(c)).astype(BF), (8, D))
    membuf[...] = _dup(mem0_ref[...].astype(F32))
    mod = _rb(_dot(sc, wms[:, pl.ds(0, CH)]))
    for i in range(2):
        modbuf[i] = _dup(mod[:, i * D:(i + 1) * D])
    fold_b(0)
    ln_pair(0)

    def fb_body(p, carry):
        cp_x(p).wait()
        for cp in cp_b(p):
            cp.wait()
        p0(p - 1, True)
        p0(NPAIR + p - 1, False)
        fold_b(p)
        ln_pair(p)
        return carry
    lax.fori_loop(1, NPAIR, fb_body, 0)

    cp_wm1.wait()
    for cp in cps_mlp:
        cp.start()
    p0(NPAIR - 1, True)
    mod = _rb(_dot(sc, wms[:, pl.ds(CH, 2 * CH)]))
    for i in range(4):
        modbuf[2 + i] = _dup(mod[:, i * D:(i + 1) * D])
    p0(NCH - 1, False)

    ga = modbuf[2][0:1]
    sb = modbuf[3][0:1]
    cb1 = _rb(1.0 + modbuf[4][0:1])
    gb = modbuf[5][0:1]
    wr = wr_ref[...].astype(F32).reshape(1, D)

    L = M + SEG
    diag = lax.broadcasted_iota(jnp.int32, (8, 128), 0) >= (lane8 % 8)
    lane40 = lax.broadcasted_iota(jnp.int32, (L, 128), 1)

    def epilogue(seg, par):
        r0 = pl.multiple_of(jnp.maximum(seg, 0) * SEG, SEG)
        attn = _rb(obuf[par])
        x = xbuf[pl.ds(r0, SEG), :]
        x2 = _rb(x + _rb(ga * attn))
        h2 = _rb(_ln_dup(x2) * cb1 + sb)
        r = _rb(jnp.sum(h2[:, :D] * wr, axis=-1, keepdims=True))
        x2buf[pl.ds(r0, SEG), :] = x2
        res = x2 + _rb(gb * h2)
        orow[0, pl.ds(r0, SEG), :] = res[:, :256]
        orow[1, pl.ds(r0, SEG), :] = res[:, 256:]
        bv = hbuf[S:S + SEG, 0:1]
        upd = jnp.logical_and(r > bv, seg >= 0)
        hbuf[S:S + SEG, 0:1] = jnp.where(upd, r, bv)
        hbuf[S + SEG:S + 2 * SEG, 0:1] = jnp.where(upd, seg.astype(F32), hbuf[S + SEG:S + 2 * SEG, 0:1])

    def out_copy(b, slot):
        return pltpu.make_async_copy(ost.at[slot, pl.ds(0, D), :],
                                     out_hbm.at[:, pl.ds(pl.multiple_of(b * 128, 128), 128)], osems.at[0])

    def trans_half(b, half, slot):
        r0 = pl.multiple_of(b * 128, 128)
        ost[slot, half * 256:(half + 1) * 256, :] = orow[half, pl.ds(r0, 128), :].T.astype(BF)

    def trans_block(b, slot):
        trans_half(b, 0, slot)
        trans_half(b, 1, slot)

    def extra_parts(s, k, half):
        b = s // 8 + 1
        is_z = half == 1
        cidx = k if is_z else NPAIR + k
        lx = _ld(hx[pl.ds(pl.multiple_of(b * 32, 32), 32), :])

        def tile(t):
            if t == 7:
                return _dot(lx[:, :D], _ld(wt2[k]))
            return proj(lx, cidx, t * 128, (t + 1) * 128)

        def finish(ts):
            y = jnp.concatenate(ts[:7], axis=1)
            for i in range(8):
                zue[b * 8 + i, cidx] = _pack_block(y[8 * i:8 * i + 8], lo_mask)
            if is_z:
                t2e[k, pl.ds(pl.multiple_of(b * 64, 64), 64), :] = ts[7]
        return tile, finish

    def step(s, par, held, k, fill1=None, fill2=None):
        with_extra = k is not None
        mem = membuf[...]
        hs = hbuf[pl.ds(pl.multiple_of(s * SEG, SEG), RIDE), :]
        lhs = jnp.concatenate([mem, hs], axis=0)[:, :D].astype(BF)
        epilogue(s - 2, par)
        hs3 = hbuf[pl.ds(pl.multiple_of(s * SEG + RIDE, 8), 8), :]
        q = jnp.concatenate([mem, hs3, hs[16:24], hs[8:16], hs[0:8]], axis=0).astype(BF)
        nrow = (40, 40, 32, 24, 16)

        def do_chunk(cidx):
            y = proj(lhs, cidx)
            for j in range(4):
                zur[j, cidx] = _pack_block(y[8 * j:8 * j + 8], lo_mask)

        def kv_tile(j, lo):
            z = zue[s, lo:lo + NPAIR] if j == 4 else zur[j, lo:lo + NPAIR]
            return _ld(z.reshape(64, DP))

        def s_tile(j):
            n16 = -(-nrow[j] // 16) * 16
            return _dot_nt(q[:min(n16, L)], kv_tile(j, 0))

        t2 = [_dot(lhs, _ld(wt2[p])) for p in range(NPAIR)]
        kb = [mem, hs[0:8], hs[8:16], hs[16:24], hs3]
        kv3 = [jnp.concatenate([jnp.where(lo_mask, k_[:, DM:], 0.0), jnp.where(lo_mask, 0.0, k_[:, DM:])],
                               axis=0).astype(BF) for k_ in kb] + [jnp.zeros((16, 128), BF)] * 3

        w3 = jnp.concatenate(kv3, axis=0)

        def tq(p):
            t3 = t2e[p, pl.ds(pl.multiple_of(s * 8, 8), 8), :]
            return [t2[p][0:8], t3, t2[p][24:32], t2[p][16:24], t2[p][8:16]]

        rs = []

        def r_tiles():
            for p in range(0, NPAIR, 2):
                r_ = _dot_nt(jnp.concatenate(tq(p) + tq(p + 1), axis=0).astype(BF), w3)
                rs.extend([pltpu.roll(r_[:L], 16 * p, 1) if p else r_[:L], pltpu.roll(r_[L:], 16 * p + 16, 1)])

        nz = NPAIR if with_extra else NPAIR + 1
        for cidx in range(nz):
            do_chunk(cidx)

        def s2_block(j, rb):
            c_ = [rs[(g - j) % 8][8 * rb:8 * rb + 8] for g in range(8)]
            for bit in (16, 32, 64):
                m_ = (lane8 & bit) != 0
                c_ = [jnp.where(m_, c_[i + 1], c_[i]) for i in range(0, len(c_), 2)]
            return pltpu.roll(c_[0], 128 - 16 * j, 1) if j else c_[0]

        tiles = [None] * 5
        if with_extra:
            etile0, efin0 = extra_parts(s, k, 0)
            ets0 = []
            for ne, j in SORD:
                ets0 += [etile0(len(ets0) + i) for i in range(ne)]
                if j == 'R':
                    r_tiles()
                else:
                    tiles[j] = s_tile(j)
            efin0(ets0)
        else:
            r_tiles()
            for j in (4, 0, 1, 2, 3):
                tiles[j] = s_tile(j)
        for cidx in range(nz, NPAIR + 7):
            do_chunk(cidx)
        blocks = []
        for j in range(5):
            nb = nrow[j] // 8
            bl = [tiles[j][8 * rb:8 * rb + 8] + s2_block(j, rb) for rb in range(nb)]
            if j >= 1:
                bl[-1] = jnp.where(diag, bl[-1], -1e9)
            blocks.append(bl)
        per_rb = lambda xs, rb: [xs[j][rb] for j in range(5) if rb < len(xs[j])]
        mx = jnp.concatenate([functools.reduce(jnp.maximum, per_rb(blocks, rb)) for rb in range(5)], axis=0)
        mx = _group_allreduce(mx, jnp.maximum, lane40)
        es = [[jnp.exp(b_ - mx[8 * rb:8 * rb + 8]) for rb, b_ in enumerate(bl)] for bl in blocks]
        sm = jnp.concatenate([functools.reduce(jnp.add, per_rb(es, rb)) for rb in range(5)], axis=0)
        sm = _group_allreduce(sm, jnp.add, lane40)
        inv = 1.0 / sm
        pf = [jnp.concatenate(es[j], axis=0) * inv[:nrow[j]] for j in range(5)]
        ps = [p_.astype(BF) for p_ in pf]
        psk = [pltpu.roll(pf[j], 16 * j, 1) if j else pf[j] for j in range(5)]
        grp = lane8 // 16

        def g_lhs(p):
            rows = []
            for rb in range(5):
                acc = jnp.zeros((8, 128), F32)
                for j in range(5):
                    if 8 * rb < nrow[j]:
                        acc = jnp.where(grp == (j + p) % 8, psk[j][8 * rb:8 * rb + 8], acc)
                rows.append(acc)
            l_ = jnp.concatenate(rows, axis=0)
            return pltpu.roll(l_, 128 - 16 * p, 1) if p else l_

        for cidx in range(NPAIR + 7, NCH):
            do_chunk(cidx)
        os_ = [None] * 5
        os_[4] = _dot(ps[4], kv_tile(4, NPAIR))
        if with_extra:
            etile, efin = extra_parts(s, k, 1)
            ets = {n: etile(n) for n in EORD[:NPRE]}
        gs = []
        for p in range(0, NPAIR, 2):
            g_ = _dot(jnp.concatenate([g_lhs(p), g_lhs(p + 1)], axis=0).astype(BF), w3)
            gs += [g_[:L], g_[L:]]
        for j in (0, 1, 2, 3):
            os_[j] = _dot(ps[j], kv_tile(j, NPAIR))
        gall = jnp.concatenate(gs, axis=1)
        if par == 0:
            held.append(gall[32:])
            gall = gall[:32]
        else:
            gall = jnp.concatenate([gall, held.pop()], axis=0)
        last = _dot(gall.astype(BF), _ld(wb2[...].reshape(NPAIR * 64, DP)))
        ob = [[os_[j][8 * rb:8 * rb + 8] for rb in range(nrow[j] // 8)] for j in range(5)]
        ob.append([last[8 * rb:8 * rb + 8] for rb in range(4 + par)])
        o = jnp.concatenate([functools.reduce(jnp.add, [b_[rb] for b_ in ob if rb < len(b_)])
                             for rb in (0, 4, 3, 2, 1)] + ([last[L:]] if par else []), axis=0)
        o3 = o[:, DM:]
        o3 = o3 + pltpu.roll(o3, 64, 1)
        o = jnp.concatenate([o[:, :DM], o3], axis=1)
        membuf[...] = o[0:M]
        obuf[par] = o[M:L]
        if par:
            obuf[0, 0:8, :] += o[L:]
        if with_extra:
            ets.update({n: etile(n) for n in EORD[NPRE:]})
            efin([ets[n] for n in range(8)])
        if fill2 is not None:
            fill1()
            fill2()

    def argmax_token():
        bv = hbuf[S:S + SEG, 0:1]
        rmax = jnp.max(bv, axis=0, keepdims=True)
        tok = hbuf[S + SEG:S + 2 * SEG, 0:1] * SEG + lax.broadcasted_iota(jnp.int32, (SEG, 1), 0).astype(F32)
        idx_f = jnp.min(jnp.where(bv == rmax, tok, float(S)), axis=0, keepdims=True)
        return jnp.clip(idx_f[0, 0].astype(jnp.int32), 0, S - 1), rmax

    def mlp_stages(idx, half):
        blk = pl.multiple_of((idx // 16) * 16, 16)
        h2b = _rb(_ln_dup(x2buf[pl.ds(blk, 16), :]) * cb1 + sb)[:, :D].astype(BF)
        st = {}
        cuts = (0, 512, CH)

        def cols(k):
            return pl.ds(pl.multiple_of(half * CH + cuts[k], 128), cuts[k + 1] - cuts[k])

        def gu(name, w, k):
            def f():
                st[name, k] = _rb(_dot(h2b, w[:, cols(k)]))
            return f

        def dn(n):
            def f():
                if n == 0:
                    g = jnp.concatenate([st['g', 0], st['g', 1]], axis=1)
                    u = jnp.concatenate([st['u', 0], st['u', 1]], axis=1)
                    st['a'] = (_rb(g * jax.nn.sigmoid(g)) * u).astype(BF)
                hc = pl.ds(pl.multiple_of(half * CH, 128), CH)
                if n < 3:
                    wl = wds[n * 128:(n + 1) * 128, hc]
                else:
                    wl = wds[DM:D, hc]
                    wl = jnp.concatenate([wl, wl], axis=0)
                spec_y[:, n * 128:(n + 1) * 128] += _dot_nt(st['a'], wl)
            return f
        return [gu('g', wgs, 0), gu('g', wgs, 1), gu('u', wus, 0), gu('u', wus, 1), dn(0), dn(1), dn(2), dn(3)]

    def body(j, k0, dma=True):
        with_extra = k0 is not None
        kk = lambda i: k0 + i if with_extra else None
        if with_extra:
            fl = [None] * 8
        else:
            fl = mlp_stages(spec_idx[0], j - 14)
        bprev = jnp.maximum(j - 1, 0)
        held = []
        step(4 * j, 0, held, kk(0), fl[0], fl[1])
        step(4 * j + 1, 1, held, kk(1), fl[2], fl[3])
        if not with_extra:
            trans_block(bprev, bprev)
        step(4 * j + 2, 0, held, kk(2), fl[4], fl[5])
        step(4 * j + 3, 1, held, kk(3), fl[6], fl[7])
        if with_extra:
            trans_block(bprev, bprev)

        if dma:
            out_copy(bprev, bprev).start()

    def body_a(j, carry):
        body(2 * j, 0, dma=False)
        body(2 * j + 1, 4, dma=False)

        @pl.when(j >= 1)
        def _():
            out_copy(2 * j - 1, 2 * j - 1).start()
        out_copy(2 * j, 2 * j).start()
        return carry
    lax.fori_loop(0, 7, body_a, 0)

    for cp in cps_mlp:
        cp.wait()
    spec_idx[0] = jnp.minimum(argmax_token()[0], 54 * SEG - 1)
    spec_y[...] = jnp.zeros((16, DP), F32)

    def body_b(j, carry):
        body(j, None)
        return carry
    lax.fori_loop(14, 16, body_b, 0)
    epilogue(jnp.int32(NSEG - 2), 0)
    epilogue(jnp.int32(NSEG - 1), 1)
    trans_block(15, 15)
    out_copy(15, 15).start()

    idx, rmax = argmax_token()

    @pl.when(idx != spec_idx[0])
    def _():
        spec_y[...] = jnp.zeros((16, DP), F32)
        for half in range(2):
            for f in mlp_stages(idx, half):
                f()

    blk = pl.multiple_of((idx // 16) * 16, 16)
    x2 = x2buf[pl.ds(blk, 16), :]
    h2 = _rb(_ln_dup(x2) * cb1 + sb)
    y = _rb(_rb(spec_y[...]) * _rb(jax.nn.sigmoid(rmax)))
    sel = lax.broadcasted_iota(jnp.int32, (16, DP), 0) == (idx - blk)
    bo = _rb(h2 + jnp.where(sel, y, 0.0))
    res = x2 + _rb(gb * bo)
    orow[0, pl.ds(blk, 16), :] = res[:, :256]
    orow[1, pl.ds(blk, 16), :] = res[:, 256:]
    fb = idx // 128
    trans_block(fb, 16)
    for b_ in range(16):
        out_copy(b_, b_).wait()
    fix = out_copy(fb, 16)
    fix.start()
    fix.wait()


@jax.jit
def pallas_adaLN_cond__memory_aug_recurrent_mem_tr__moe_arch_mod__prompt_kernel(A_x, A_mem0, A_Wq, A_Wk, A_Wv, A_Wo, A_seg_len, B_x, B_w_r, B_w_gate, B_w_up, B_w_down, c, w_mod):
    hbm = pl.BlockSpec(memory_space=pltpu.HBM)
    out = pl.pallas_call(
        _kernel,
        out_shape=jax.ShapeDtypeStruct((D, S), BF),
        in_specs=[hbm] * 12,
        out_specs=hbm,
        scratch_shapes=[
            pltpu.VMEM((8, D, 256), BF),
            pltpu.VMEM((NPAIR, D, E), jnp.uint32),
            pltpu.VMEM((NPAIR, D, E), jnp.uint32),
            pltpu.VMEM((NPAIR, D, E), jnp.uint32),
            pltpu.VMEM((NPAIR, CH, E), BF),
            pltpu.VMEM((D, F), BF),
            pltpu.VMEM((D, F), BF),
            pltpu.VMEM((D, F), BF),
            pltpu.VMEM((D, 6 * D), BF),
            pltpu.VMEM((NCH, DM // 2, CH), jnp.uint32),
            pltpu.VMEM((NPAIR, D // 2, 128), jnp.uint32),
            pltpu.VMEM((NPAIR, 64, DP), jnp.uint32),
            pltpu.VMEM((NPAIR, NSEG * 8, 128), F32),
            pltpu.VMEM((S + 2 * SEG, DP), F32),
            pltpu.VMEM((S, DP), F32),
            pltpu.VMEM((NSEG * 4, DP), jnp.uint32),
            pltpu.VMEM((4, NCH, 8, DP), jnp.uint32),
            pltpu.VMEM((NSEG, NCH, 8, DP), jnp.uint32),
            pltpu.VMEM((M, DP), F32),
            pltpu.VMEM((2, SEG, DP), F32),
            pltpu.VMEM((S, DP), F32),
            pltpu.VMEM((2, S, 256), F32),
            pltpu.VMEM((6, 8, DP), F32),
            pltpu.VMEM((17, DP, 128), BF),
            pltpu.VMEM((16, DP), F32),
            pltpu.VMEM((M, D), BF),
            pltpu.VMEM((D,), BF),
            pltpu.VMEM((1, D), BF),
            pltpu.SMEM((1,), jnp.int32),
            pltpu.SemaphoreType.DMA((NCH,)),
            pltpu.SemaphoreType.DMA((2,)),
            pltpu.SemaphoreType.DMA((1,)),
        ],
        compiler_params=pltpu.CompilerParams(vmem_limit_bytes=110 * 1024 * 1024),
    )(A_x.reshape(S, D).T, A_mem0.reshape(M, D), A_Wq, A_Wk, A_Wv,
      jnp.transpose(A_Wo, (0, 2, 1)).reshape(NPAIR, CH, E), B_w_r,
      B_w_gate, B_w_up, B_w_down.T, c, w_mod)
    return out.T.reshape(1, S, D)
```
